```python
import os as _os
_os.environ.setdefault("JAX_PLATFORMS", "cpu")
import jax
import jax.numpy as jnp

def _softmax(x, axis=-1):
    return jax.nn.softmax(x, axis=axis)
def _gelu(x):
    return jax.nn.gelu(x, approximate=True)
def _silu(x):
    return jax.nn.silu(x)
def _sigmoid(x):
    return jax.nn.sigmoid(x)
def _layernorm(x, axis=-1, eps=1e-5):
    m = jnp.mean(x, axis=axis, keepdims=True)
    v = jnp.var(x, axis=axis, keepdims=True)
    return (x - m) / jnp.sqrt(v + eps)
def _scatter_add(tgt, idx, src, axis=0):
    return tgt.at[idx].add(src)
def _segment_sum(src, seg, n):
    return jax.ops.segment_sum(src, seg, n)
class _Rng:
    def __init__(self, key):
        self._k = key
    def _next(self):
        self._k, sub = jax.random.split(self._k)
        return sub
    def normal(self, shape):
        return jax.random.normal(self._next(), shape, dtype=jnp.bfloat16)
    def randint(self, lo, hi, shape):
        return jax.random.randint(self._next(), shape, lo, hi, dtype=jnp.int32)
    def uniform(self, shape, lo=0.0, hi=1.0):
        return jax.random.uniform(self._next(), shape, jnp.bfloat16, lo, hi)
    def permutation(self, n):
        return jax.random.permutation(self._next(), n)


kernel_name = 'standalone__channel_attn_cbam__vision'

def setup_inputs():
    _rng = _Rng(jax.random.key(int.from_bytes(__import__("os").urandom(4), "little")))
    _w = (lambda a: (lambda t: t.astype(jnp.bfloat16) if jnp.issubdtype(t.dtype, jnp.floating) else t)(jnp.asarray(a)))
    H = W = 224
    C = 192
    r = max(C // 4, 1)
    return {
        "x": _w((lambda *s: _rng.normal(s) * 0.2)(1, H, W, C) + (lambda *s: _rng.normal(s) * 0.2)(1, 1, 1, C) * 2.0),
        "w1": _w((lambda *s: _rng.normal(s) * 0.2)(C, r)),
        "w2": _w((lambda *s: _rng.normal(s) * 0.2)(r, C)),
    }

def reference(x, w1, w2):
    B, H, W, C = x.shape
    xf = x.reshape(B, H * W, C)
    gap = jnp.mean(xf, 1)
    gmp = jnp.amax(xf, 1)
    h_a = gap @ w1
    h_a = h_a * (lambda x, dt: x.astype(dt))(h_a > 0, h_a.dtype)
    h_m = gmp @ w1
    h_m = h_m * (lambda x, dt: x.astype(dt))(h_m > 0, h_m.dtype)
    scale = _sigmoid(h_a @ w2 + h_m @ w2)
    return x * scale[:, None, None, :]
```

```python
import jax
import jax.numpy as jnp
from jax import lax
import jax.experimental.pallas as pl
import jax.experimental.pallas.tpu as pltpu

_LANES = 128
_BLK = 32
_S = 2048
_P = 3
_BPS = _S // _BLK
_BPU = _P * _BPS
_LAST_BLOCKS = 18
_NSEM = 2


def _kernel(x_hbm, w1t_hbm, w2_hbm, o_hbm,
            buf, w1t_v, w2_v, w1c, w2c, acc_s, acc_m, scale_v, sem):
    NU, _, _, W = buf.shape
    R, C = w1t_v.shape
    G = C // _BLK
    NB = NU * _BPU
    N = NB // G * W
    half = _LANES // 2

    bounds = (0, NB - 2 * _BPU, NB - _BPU, NB - _BPS, NB - _LAST_BLOCKS, NB)
    boxes = (
        (pl.ds(0, NU - 2),),
        (pl.ds(NU - 2, 1),),
        (NU - 1, pl.ds(0, _P - 1)),
        (NU - 1, _P - 1, pl.ds(0, _S - _LAST_BLOCKS * _BLK)),
        (NU - 1, _P - 1, pl.ds(_S - _LAST_BLOCKS * _BLK, _LAST_BLOCKS * _BLK)),
    )
    reads = [
        pltpu.make_async_copy(x_hbm.at[box], buf.at[box], sem.at[i % _NSEM])
        for i, box in enumerate(boxes)
    ]
    w_reads = [
        pltpu.make_async_copy(w1t_hbm, w1t_v, sem.at[0]),
        pltpu.make_async_copy(w2_hbm, w2_v, sem.at[0]),
    ]
    for c in reads[:_NSEM]:
        c.start(priority=1)
    for c in w_reads:
        c.start()

    def wait_read(i):
        reads[i].wait()
        if i == 0:
            for c in w_reads:
                c.wait()
        if i + _NSEM < len(reads):
            reads[i + _NSEM].start(priority=1)

    def pool(b0, b1, g):
        def run(u, l0, l1, carry):
            for l in range(l0, l1, G):
                if isinstance(g, int):
                    a, r0 = (l + g) // _BPS, (l + g) % _BPS * _BLK
                else:
                    a = lax.shift_right_logical(l + g, _BPS.bit_length() - 1)
                    r0 = pl.multiple_of(
                        lax.bitwise_and(l + g, _BPS - 1) * _BLK, _BLK)
                v = buf[u, a, pl.ds(r0, _BLK), :].astype(jnp.float32)
                if carry is None:
                    carry = (v, v)
                else:
                    carry = (carry[0] + v, jnp.maximum(carry[1], v))
            return carry

        if b1 - b0 > _BPU:
            init = (jnp.zeros((_BLK, W), jnp.float32),
                    jnp.full((_BLK, W), -jnp.inf, jnp.float32))
            s, m = lax.fori_loop(b0 // _BPU, b1 // _BPU,
                                 lambda u, c: run(u, 0, _BPU, c), init)
        else:
            u = b0 // _BPU
            s, m = run(u, b0 - u * _BPU, b1 - u * _BPU, None)
        valid = lax.broadcasted_iota(jnp.int32, (_BLK, _LANES), 1) < W - _LANES
        pad = ((0, 0), (0, 2 * _LANES - W))
        s = s[:, :_LANES] + jnp.where(valid, jnp.pad(s[:, _LANES:], pad), 0.0)
        m = jnp.maximum(
            m[:, :_LANES],
            jnp.where(valid, jnp.pad(m[:, _LANES:], pad), -jnp.inf))
        return s, m

    done = [b // G * G for b in bounds]
    for i in range(len(reads) - 1):
        wait_read(i)
        if i == 0:
            zeros = jnp.zeros((half - R, C), jnp.float32)
            for src, dst in ((w1t_v, w1c), (w2_v, w2c)):
                w = src[...].astype(jnp.float32)
                dst[...] = jnp.concatenate([w, zeros, w, zeros], axis=0).T

        def pool_group(g, carry, i=i):
            cs = pl.ds(pl.multiple_of(g * _BLK, _BLK), _BLK)
            s, m = pool(done[i], done[i + 1], g)
            if i > 0:
                s = s + acc_s[cs, :]
                m = jnp.maximum(m, acc_m[cs, :])
            acc_s[cs, :] = s
            acc_m[cs, :] = m
            return carry

        lax.fori_loop(0, G, pool_group, None)

    wait_read(len(reads) - 1)
    avg_lane = lax.broadcasted_iota(jnp.int32, (_BLK, _LANES), 1) < half
    h = None
    for g in range(G):
        cs = pl.ds(g * _BLK, _BLK)
        s, m = pool(done[-2], done[-1], g)
        gap = jnp.sum(s + acc_s[cs, :], axis=1, keepdims=True) * (1.0 / N)
        gmp = jnp.max(jnp.maximum(m, acc_m[cs, :]), axis=1, keepdims=True)
        prod = jnp.where(avg_lane, gap, gmp) * w1c[cs, :]
        for k in range(0, _BLK, 8):
            h = prod[k:k + 8] if h is None else h + prod[k:k + 8]
    h = jnp.sum(h, axis=0, keepdims=True)
    used = (lax.broadcasted_iota(jnp.int32, (1, _LANES), 1) & (half - 1)) < R
    h = jnp.where(used, h * (h > 0).astype(jnp.float32), 0.0)

    order = [(q * _BPS) % G for q in range(_P)]
    order += [g for g in range(G) if g not in order]
    logit = {
        g: jnp.broadcast_to(
            jnp.sum(w2c[pl.ds(g * _BLK, _BLK), :] * h, axis=1, keepdims=True),
            (_BLK, _LANES))
        for g in order
    }

    def rescale(q, r0, scale):
        scale = jnp.concatenate([scale, scale], axis=1)[:, :W]
        for u in range(NU):
            v = buf[u, q, pl.ds(r0, _BLK), :].astype(jnp.float32)
            buf[u, q, pl.ds(r0, _BLK), :] = (v * scale).astype(buf.dtype)

    def write(box):
        pltpu.make_async_copy(buf.at[box], o_hbm.at[box], sem.at[0]).start()

    scale0 = jax.nn.sigmoid(logit[0])
    rescale(0, 0, scale0)
    write((slice(None), 0, pl.ds(0, _BLK)))
    scale_v[pl.ds(0, _BLK), :] = scale0
    for g in range(1, G):
        scale_v[pl.ds(g * _BLK, _BLK), :] = logit[g]

    def first_block(q, carry):
        cs = pl.ds(pl.multiple_of(lax.rem(q * _BPS, G) * _BLK, _BLK), _BLK)
        scale = jax.nn.sigmoid(scale_v[cs, :])
        scale_v[cs, :] = scale
        rescale(q, 0, scale)
        write((slice(None), q, pl.ds(0, _BLK)))
        return carry

    lax.fori_loop(1, _P, first_block, None)
    for g in order[_P:]:
        cs = pl.ds(g * _BLK, _BLK)
        scale_v[cs, :] = jax.nn.sigmoid(scale_v[cs, :])

    def row_block(j, carry):
        r0 = pl.multiple_of(j * _BLK, _BLK)
        for q in range(_P):
            c0 = pl.multiple_of(lax.rem(j + q * _BPS, G) * _BLK, _BLK)
            rescale(q, r0, scale_v[pl.ds(c0, _BLK), :])
        write((slice(None), slice(None), pl.ds(r0, _BLK)))
        return carry

    lax.fori_loop(1, _BPS, row_block, None)
    pltpu.make_async_copy(buf, o_hbm, sem.at[0]).wait()


@jax.jit
def pallas_standalone__channel_attn_cbam__vision_kernel(
    x: jax.Array,
    w1: jax.Array,
    w2: jax.Array,
):
    B, H, W, C = x.shape
    R = w1.shape[1]
    G = C // _BLK
    assert B == 1 and _LANES < W <= 2 * _LANES and R <= _LANES // 2
    assert C % _BLK == 0 and _BPU % G == 0 and _LAST_BLOCKS % G == 0
    assert len({(q * _BPS) % G for q in range(_P)}) == _P
    assert (H * C) % (_P * _S) == 0 and H * C // (_P * _S) >= 4
    shape = (H * C // (_P * _S), _P, _S, W)

    xt = jnp.transpose(x, (0, 1, 3, 2)).reshape(shape)
    out = pl.pallas_call(
        _kernel,
        in_specs=[pl.BlockSpec(memory_space=pl.ANY)] * 3,
        out_specs=pl.BlockSpec(memory_space=pl.ANY),
        out_shape=jax.ShapeDtypeStruct(shape, x.dtype),
        scratch_shapes=[
            pltpu.VMEM(shape, x.dtype),
            pltpu.VMEM((R, C), w1.dtype),
            pltpu.VMEM((R, C), w2.dtype),
            pltpu.VMEM((C, _LANES), jnp.float32),
            pltpu.VMEM((C, _LANES), jnp.float32),
            pltpu.VMEM((C, _LANES), jnp.float32),
            pltpu.VMEM((C, _LANES), jnp.float32),
            pltpu.VMEM((C, _LANES), jnp.float32),
            pltpu.SemaphoreType.DMA((_NSEM,)),
        ],
        compiler_params=pltpu.CompilerParams(vmem_limit_bytes=64 * 1024 * 1024),
    )(xt, w1.T, w2)
    return jnp.transpose(out.reshape(B, H, C, W), (0, 1, 3, 2))
```
